```python
import os as _os
_os.environ.setdefault("JAX_PLATFORMS", "cpu")
import jax
import jax.numpy as jnp

def _softmax(x, axis=-1):
    return jax.nn.softmax(x, axis=axis)
def _gelu(x):
    return jax.nn.gelu(x, approximate=True)
def _silu(x):
    return jax.nn.silu(x)
def _sigmoid(x):
    return jax.nn.sigmoid(x)
def _layernorm(x, axis=-1, eps=1e-5):
    m = jnp.mean(x, axis=axis, keepdims=True)
    v = jnp.var(x, axis=axis, keepdims=True)
    return (x - m) / jnp.sqrt(v + eps)
def _scatter_add(tgt, idx, src, axis=0):
    return tgt.at[idx].add(src)
def _segment_sum(src, seg, n):
    return jax.ops.segment_sum(src, seg, n)
class _Rng:
    def __init__(self, key):
        self._k = key
    def _next(self):
        self._k, sub = jax.random.split(self._k)
        return sub
    def normal(self, shape):
        return jax.random.normal(self._next(), shape, dtype=jnp.bfloat16)
    def randint(self, lo, hi, shape):
        return jax.random.randint(self._next(), shape, lo, hi, dtype=jnp.int32)
    def uniform(self, shape, lo=0.0, hi=1.0):
        return jax.random.uniform(self._next(), shape, jnp.bfloat16, lo, hi)
    def permutation(self, n):
        return jax.random.permutation(self._next(), n)


kernel_name = 'sequential_preLN__mha_block__moe_arch_mod__prompt'

def setup_inputs():
    _rng = _Rng(jax.random.key(int.from_bytes(__import__("os").urandom(4), "little")))
    _w = (lambda a: (lambda t: t.astype(jnp.bfloat16) if jnp.issubdtype(t.dtype, jnp.floating) else t)(jnp.asarray(a)))
    def _A_setup():
        B, S, D, H = 1, 2048, 640, 32
        return {
            "x": _w((lambda *s: _rng.normal(s) * 0.05)(B, S, D)),
            "wqkv": _w((lambda *s: _rng.normal(s) * 0.05)(D, 3 * D)),
            "wo": _w((lambda *s: _rng.normal(s) * 0.05)(D, D)),
        }
    _A_in = _A_setup()

    def _B_setup():
        B, S, D, F, C = 1, 2048, 640, 1536, 1
        return {
            "x": _w((lambda *s: _rng.normal(s) * 0.05)(B, S, D)),
            "w_r": _w((lambda *s: _rng.normal(s) * 0.05)(D)),
            "w_gate": _w((lambda *s: _rng.normal(s) * 0.05)(D, F)),
            "w_up": _w((lambda *s: _rng.normal(s) * 0.05)(D, F)),
            "w_down": _w((lambda *s: _rng.normal(s) * 0.05)(F, D)),
        }
    _B_in = _B_setup()

    return {
        "A_x": _A_in["x"],
        "A_wqkv": _A_in["wqkv"],
        "A_wo": _A_in["wo"],
        "B_x": _B_in["x"],
        "B_w_r": _B_in["w_r"],
        "B_w_gate": _B_in["w_gate"],
        "B_w_up": _B_in["w_up"],
        "B_w_down": _B_in["w_down"],
    }

def reference(A_x, A_wqkv, A_wo, B_x, B_w_r, B_w_gate, B_w_up, B_w_down):
    def _A_ref(x, wqkv, wo):
        B, S, D = x.shape
        H = 32
        Dh = D // H
        qkv = (lambda x, *d: x.transpose(*d))((x @ wqkv).reshape(B, S, 3, H, Dh), 2, 0, 3, 1, 4)
        q, k, v = qkv[0], qkv[1], qkv[2]
        scores = jnp.einsum("bhqd,bhkd->bhqk", q, k) * (Dh ** -0.5)
        p = _softmax(scores, axis=-1)
        o = jnp.einsum("bhqk,bhkd->bhqd", p, v)
        return (lambda x, *d: x.transpose(*d))(o, 0, 2, 1, 3).reshape(B, S, D) @ wo

    def _B_ref(x, w_r, w_gate, w_up, w_down):
        B, S, D = x.shape
        C = 1
        r = x @ w_r
        idx = jnp.argsort(-r, axis=-1)[:, :C]
        idx_e = jnp.repeat(idx.reshape(B, C, 1), D, axis=2)
        x_sel = jnp.take_along_axis(x, idx_e, axis=1)
        g = _silu(x_sel @ w_gate)
        u = x_sel @ w_up
        y = (g * u) @ w_down
        r_sel = _sigmoid(jnp.take_along_axis(r, idx, axis=1))
        y = y * r_sel.reshape(B, C, 1)
        b_off = (jnp.arange(B) * S).reshape(B, 1)
        flat_idx = (idx + b_off).reshape(B * C)
        zero = (x * 0.0).reshape(B * S, D)
        upd = _scatter_add(zero, flat_idx, y.reshape(B * C, D), axis=0)
        return x + upd.reshape(B, S, D)

    x = A_x
    h = x + _A_ref(_layernorm(x, axis=-1), A_wqkv, A_wo)
    h2 = h + _B_ref(_layernorm(h, axis=-1), B_w_r, B_w_gate, B_w_up, B_w_down)
    return h2
```

```python
import functools
import math

import numpy as np
import jax
import jax.numpy as jnp
from jax import lax
import jax.experimental.pallas as pl
import jax.experimental.pallas.tpu as pltpu

S, D, H, DH, F = 2048, 640, 32, 20, 1536
WIN = (0, 120, 240, 360, 480, 512)
QK_SCALE = float(DH ** -0.5 * math.log2(math.e))
LN_EPS = 1e-5
L_LO, L_HI = 2.0 ** -60, 2.0 ** 100
BIG = 3.0e38

VR = 24

NT = (((1,), (1,)), ((), ()))
NN = (((1,), (0,)), ((), ()))
TN = (((0,), (0,)), ((), ()))


def _ln(xf):
    m = jnp.mean(xf, axis=-1, keepdims=True)
    c = xf - m
    v = jnp.mean(c * c, axis=-1, keepdims=True)
    return c * lax.rsqrt(v + LN_EPS)


def make_kernel(KC=128, NQ=512, NQB=4, DEPTH=1, RB=256, EB=256, interpret=False, flags=None, scopes=False):
    nc = S // KC
    ngrp = S // (NQ * NQB)

    def scope(name):
        return jax.named_scope(name)

    def kernel(x_ref, wqkv_ref, wo_ref, wr_ref, wg_hbm, wu_hbm, wd_hbm, out_ref,
               ln1_s, wt_s, wk_s, kp_s, qt_s, vt_s, ot_s, ln2_s, hb_s, r_s, wg_s, wu_s, wd_s, sems):
        cp_g = pltpu.make_async_copy(wg_hbm, wg_s, sems.at[0])
        cp_u = pltpu.make_async_copy(wu_hbm, wu_s, sems.at[1])
        cp_d = pltpu.make_async_copy(wd_hbm, wd_s, sems.at[2])
        cp_g.start()
        cp_u.start()
        cp_d.start()

        with scope("ln1"):
            def ln1_body(i, c):
                r0 = pl.multiple_of(i * RB, RB)
                xf = x_ref[pl.ds(r0, RB), :].astype(jnp.float32)
                ln1_s[pl.ds(r0, RB), :] = _ln(xf).astype(jnp.bfloat16)
                return c
            lax.fori_loop(0, S // RB, ln1_body, 0)

        with scope("wprep"):
            wt_s[0:D, :] = wqkv_ref[:, 0:D].T
            wt_s[D:2 * D, :] = wqkv_ref[:, 2 * D:3 * D].T
            for g in range(6):
                c0 = D + WIN[g]
                wk_s[:, g * 128:(g + 1) * 128] = wqkv_ref[:, c0:c0 + 128]

        with scope("proj"):
            def proj_body(i, c):
                t0 = pl.multiple_of(i * 512, 512)
                lb = ln1_s[pl.ds(t0, 512), :]
                kk = jnp.dot(lb, wk_s[...], preferred_element_type=jnp.float32)
                for g in range(6):
                    kp_s[g, pl.ds(t0, 512), :] = kk[:, g * 128:(g + 1) * 128].astype(jnp.bfloat16)
                qt = lax.dot_general(wt_s[0:D, :], lb, NT, preferred_element_type=jnp.float32)
                qt_s[:, pl.ds(t0, 512)] = qt * QK_SCALE
                vt = lax.dot_general(wt_s[D:2 * D, :], lb, NT, preferred_element_type=jnp.float32)
                vt_s[:, pl.ds(t0, 512)] = vt.astype(jnp.bfloat16).astype(jnp.float32)
                return c
            lax.fori_loop(0, S // 512, proj_body, 0)

        def head_geom(h):
            g = h // 6
            wq0 = pl.multiple_of(jnp.minimum(g * 120, 512), 8)
            off_q = h * DH - wq0
            w0 = pl.multiple_of((h * DH // 8) * 8, 8)
            off_v = h * DH - w0
            return g, wq0, off_q, w0, off_v

        def fold(b, n):
            b = b[0:8] + b[8:16] + b[16:24]
            r = b[:, 0:128]
            for i in range(1, n // 128):
                r = r + b[:, i * 128:(i + 1) * 128]
            return r

        def finish(acc, off_v, w0, q0, n):
            row = lax.broadcasted_iota(jnp.int32, (VR, n), 0)
            vm = (row >= off_v) & (row < off_v + DH)
            l = jnp.max(jnp.where(vm, 0.0, acc), axis=0, keepdims=True)
            l = jnp.where(jnp.isfinite(jnp.sum(jnp.where(vm, 0.0, acc), axis=0, keepdims=True)), l, jnp.nan)
            o = acc * (1.0 / l)
            pltpu.store(ot_s.at[pl.ds(w0, VR), pl.ds(q0, n)], o, mask=vm)
            return o, l

        def fast_body(i, flag):
            h = i // ngrp
            jg = i % ngrp
            g, wq0, off_q, w0, off_v = head_geom(h)
            rowq = lax.broadcasted_iota(jnp.int32, (128, NQ), 0)
            qmask = (rowq >= off_q) & (rowq < off_q + DH)
            rowv = lax.broadcasted_iota(jnp.int32, (VR, KC), 0)
            vmask = (rowv >= off_v) & (rowv < off_v + DH)
            qms = {}

            def q0_of(j):
                return pl.multiple_of((jg * NQB + j) * NQ, NQ)

            def get_qm(j):
                if j not in qms:
                    q = qt_s[pl.ds(wq0, 128), pl.ds(q0_of(j), NQ)]
                    qms[j] = jnp.where(qmask, q, 0.0).astype(jnp.bfloat16)
                return qms[j]

            def qk(j, c):
                return jnp.dot(kp_s[g, pl.ds(c * KC, KC), :], get_qm(j), preferred_element_type=jnp.float32)

            def pv(c, p):
                v = jnp.where(vmask, vt_s[pl.ds(w0, VR), pl.ds(c * KC, KC)], 1.0)
                return lax.dot_general(v, p, NN, preferred_element_type=jnp.float32)

            steps = [(j, c) for j in range(NQB) for c in range(nc)]
            n = len(steps)
            ps, accs = {}, {}
            for t in range(min(DEPTH, n)):
                ps[t] = jnp.exp2(qk(*steps[t])).astype(jnp.bfloat16)
            for t in range(n):
                if t + DEPTH < n:
                    s = qk(*steps[t + DEPTH])
                j, c = steps[t]
                r = pv(c, ps.pop(t))
                accs[j] = r if c == 0 else accs[j] + r
                if t + DEPTH < n:
                    ps[t + DEPTH] = jnp.exp2(s).astype(jnp.bfloat16)
                if c == nc - 1:
                    o, l = finish(accs.pop(j), off_v, w0, q0_of(j), NQ)
                    ok = (jnp.abs(o) <= BIG) & (l >= L_LO) & (l <= L_HI)
                    flag = flag + fold(jnp.where(ok, 0.0, 1.0), NQ)
            return flag

        with scope("attn_fast"):
            flag = lax.fori_loop(0, H * ngrp, fast_body, jnp.zeros((8, 128), jnp.float32))

        unsafe = jnp.max(flag) > 0.0

        @pl.when(unsafe)
        def _():
            SQ, SK = 512, 256

            def slow_body(i, c0):
                h = i // (S // SQ)
                j = i % (S // SQ)
                g, wq0, off_q, w0, off_v = head_geom(h)
                q0 = pl.multiple_of(j * SQ, SQ)
                rowq = lax.broadcasted_iota(jnp.int32, (128, SQ), 0)
                qmask = (rowq >= off_q) & (rowq < off_q + DH)
                rowv = lax.broadcasted_iota(jnp.int32, (VR, SK), 0)
                vmask = (rowv >= off_v) & (rowv < off_v + DH)
                qm = jnp.where(qmask, qt_s[pl.ds(wq0, 128), pl.ds(q0, SQ)], 0.0).astype(jnp.bfloat16)

                def c_body(c, carry):
                    m, acc = carry
                    k0 = pl.multiple_of(c * SK, SK)
                    s = jnp.dot(kp_s[g, pl.ds(k0, SK), :], qm, preferred_element_type=jnp.float32)
                    mn = jnp.maximum(m, jnp.max(s, axis=0, keepdims=True))
                    p = jnp.exp2(s - mn).astype(jnp.bfloat16)
                    alpha = jnp.exp2(m - mn)
                    v = jnp.where(vmask, vt_s[pl.ds(w0, VR), pl.ds(k0, SK)], 1.0)
                    acc = acc * alpha + lax.dot_general(v, p, NN, preferred_element_type=jnp.float32)
                    return mn, acc
                m, acc = lax.fori_loop(0, S // SK, c_body,
                                       (jnp.full((1, SQ), -jnp.inf, jnp.float32), jnp.zeros((VR, SQ), jnp.float32)))
                finish(acc, off_v, w0, q0, SQ)
                return c0
            lax.fori_loop(0, H * (S // SQ), slow_body, 0)

        with scope("epi"):
            def epi_body(i, c):
                r0 = pl.multiple_of(i * EB, EB)
                ot = ot_s[:, pl.ds(r0, EB)].astype(jnp.bfloat16)
                a = lax.dot_general(ot, wo_ref[...], TN, preferred_element_type=jnp.float32)
                hh = x_ref[pl.ds(r0, EB), :].astype(jnp.float32) + a
                l2 = _ln(hh)
                l2b = l2.astype(jnp.bfloat16)
                ln2_s[pl.ds(r0, EB), :] = l2b
                hb = hh + l2
                hb_s[pl.ds(r0, EB), :] = hb
                out_ref[pl.ds(r0, EB), :] = hb.astype(jnp.bfloat16)
                rr = jnp.sum(l2b.astype(jnp.float32) * wr_ref[...].astype(jnp.float32), axis=-1, keepdims=True)
                r_s[pl.ds(r0, EB), :] = rr
                return c
            lax.fori_loop(0, S // EB, epi_body, 0)

        with scope("route"):
            rb = r_s[...].astype(jnp.bfloat16).astype(jnp.float32)
            rk = jnp.where(rb != rb, -jnp.inf, rb)
            best = jnp.max(rk, axis=0, keepdims=True)
            ids = lax.broadcasted_iota(jnp.int32, (S, 1), 0)
            idx_v = jnp.min(jnp.where(rk == best, ids, S - 1), axis=0, keepdims=True)
            r_sel = jnp.max(jnp.where(ids == idx_v, rb, -jnp.inf), axis=0, keepdims=True)
            idx = idx_v[0, 0]
            base = pl.multiple_of((idx // 16) * 16, 16)
            sel = lax.broadcasted_iota(jnp.int32, (16, D), 0) == (idx - base)
            tile = ln2_s[pl.ds(base, 16), :].astype(jnp.float32)
            xs = jnp.sum(jnp.where(sel, tile, 0.0), axis=0, keepdims=True)
            xs16 = jnp.broadcast_to(xs, (16, D)).astype(jnp.bfloat16)
            cp_g.wait()
            cp_u.wait()
            cp_d.wait()
            gg = jnp.dot(xs16, wg_s[...], preferred_element_type=jnp.float32).astype(jnp.bfloat16).astype(jnp.float32)
            uu = jnp.dot(xs16, wu_s[...], preferred_element_type=jnp.float32).astype(jnp.bfloat16).astype(jnp.float32)
            act = (gg * jax.nn.sigmoid(gg)).astype(jnp.bfloat16).astype(jnp.float32)
            gu = (act * uu).astype(jnp.bfloat16)
            y = jnp.dot(gu, wd_s[...], preferred_element_type=jnp.float32)
            y = y * jax.nn.sigmoid(r_sel)
            hb = hb_s[pl.ds(base, 16), :]
            out_ref[pl.ds(base, 16), :] = jnp.where(sel, hb + y, hb).astype(jnp.bfloat16)

    def call(x, wqkv, wo, wr, wg, wu, wd):
        vm = pl.BlockSpec(memory_space=pltpu.VMEM)
        anym = pl.BlockSpec(memory_space=pl.ANY)
        cp = dict(vmem_limit_bytes=100 * 2 ** 20)
        if flags:
            cp["flags"] = flags
        return pl.pallas_call(
            kernel,
            out_shape=jax.ShapeDtypeStruct((S, D), jnp.bfloat16),
            in_specs=[vm, vm, vm, vm, anym, anym, anym],
            out_specs=vm,
            scratch_shapes=[
                pltpu.VMEM((S, D), jnp.bfloat16),
                pltpu.VMEM((2 * D, D), jnp.bfloat16),
                pltpu.VMEM((D, 768), jnp.bfloat16),
                pltpu.VMEM((6, S, 128), jnp.bfloat16),
                pltpu.VMEM((D, S), jnp.float32),
                pltpu.VMEM((D, S), jnp.float32),
                pltpu.VMEM((D, S), jnp.float32),
                pltpu.VMEM((S, D), jnp.bfloat16),
                pltpu.VMEM((S, D), jnp.float32),
                pltpu.VMEM((S, 1), jnp.float32),
                pltpu.VMEM((D, F), jnp.bfloat16),
                pltpu.VMEM((D, F), jnp.bfloat16),
                pltpu.VMEM((F, D), jnp.bfloat16),
                pltpu.SemaphoreType.DMA((3,)),
            ],
            compiler_params=pltpu.CompilerParams(**cp),
            interpret=interpret,
            name="mha_mod_block",
        )(x, wqkv, wo, wr, wg, wu, wd)

    @jax.jit
    def fn(A_x, A_wqkv, A_wo, B_x, B_w_r, B_w_gate, B_w_up, B_w_down):
        out = call(A_x.reshape(S, D), A_wqkv, A_wo, B_w_r.reshape(1, D), B_w_gate, B_w_up, B_w_down)
        return out.reshape(1, S, D)

    return fn


_fn = make_kernel(NQ=512, NQB=4)


@jax.jit
def pallas_sequential_preLN__mha_block__moe_arch_mod__prompt_kernel(
    A_x: jax.Array,
    A_wqkv: jax.Array,
    A_wo: jax.Array,
    B_x: jax.Array,
    B_w_r: jax.Array,
    B_w_gate: jax.Array,
    B_w_up: jax.Array,
    B_w_down: jax.Array,
):
    return _fn(A_x, A_wqkv, A_wo, B_x, B_w_r, B_w_gate, B_w_up, B_w_down)
```

```python
import math

import jax
import jax.numpy as jnp
from jax import lax
import jax.experimental.pallas as pl
import jax.experimental.pallas.tpu as pltpu

S, D, H, DH, F = 2048, 640, 32, 20, 1536
ND = D // 128
QK_SCALE = float(DH ** -0.5 * math.log2(math.e))
LN_EPS = 1e-5
L_LO, L_HI = 2.0 ** -40, 2.0 ** 100
BIG = 3.0e38

SPECIAL = ((6, 0), (12, 24), (19, 52), (25, 76))

VR = 24
KC = 256
NQ = 512
HPB = 2
TAIL = 3
TB = 256
NSMALL = 3
PB = 512
EB = 128
OB = 512

NT = (((1,), (1,)), ((), ()))
NN = (((1,), (0,)), ((), ()))
TN = (((0,), (0,)), ((), ()))
F32, BF16, U32 = jnp.float32, jnp.bfloat16, jnp.uint32


def _ln(xf):
    m = jnp.mean(xf, axis=-1, keepdims=True)
    c = xf - m
    v = jnp.mean(c * c, axis=-1, keepdims=True)
    return c * lax.rsqrt(v + LN_EPS)


def _cat(parts):
    return jnp.concatenate(parts, axis=1)


def _round(v):
    return v.astype(BF16).astype(F32)


def _pack(v):
    return pltpu.bitcast(v, U32)


def _unpack(v):
    return pltpu.bitcast(v, BF16)


def _rows(start, size, align):
    return pl.ds(start if isinstance(start, int) else pl.multiple_of(start, align), size)


def _head_geom(h):
    kt = (h * DH) // 128
    wq0 = kt * 128
    for hs, lane in SPECIAL:
        kt = jnp.where(h == hs, ND, kt)
        wq0 = jnp.where(h == hs, hs * DH - lane, wq0)
    wq0 = pl.multiple_of(wq0, 8)
    w0 = pl.multiple_of(((h * DH) // 8) * 8, 8)
    return kt, wq0, h * DH - wq0, w0, h * DH - w0


def _row_mask(shape, lo):
    row = lax.broadcasted_iota(jnp.int32, shape, 0)
    return (row >= lo) & (row < lo + DH)


def _kernel(x_hbm, wqkv_hbm, wo_hbm, wr_hbm, wg_hbm, wu_hbm, wd_hbm, out_hbm,
            x_s, w_s, wo_s, wr_s, wg_s, wu_s, wd_s, out_s, fix_s,
            ln1_s, wt_s, k_s, qt_s, vt_s, ot_s, ln2_s,
            sem_x, sem_w, sem_f, sem_o):
    x_pieces = [(i * TB, TB) for i in range(NSMALL)] + [(NSMALL * TB, S - NSMALL * TB)]
    cp_x = [pltpu.make_async_copy(x_hbm.at[pl.ds(r0, n), :], x_s.at[pl.ds(r0, n), :], sem_x.at[i])
            for i, (r0, n) in enumerate(x_pieces)]

    def start_slabs(src, col0, dst, slab0, sem):
        for j in range(ND):
            pltpu.make_async_copy(src.at[:, pl.ds(col0 + j * 128, 128)], dst.at[slab0 + j], sem).start()

    def wait_slabs(dst, slab0, sem):
        v = dst.at[pl.ds(slab0, ND)]
        pltpu.make_async_copy(v, v, sem).wait()

    cp_wr = pltpu.make_async_copy(wr_hbm, wr_s, sem_w.at[4])
    cp_g = pltpu.make_async_copy(wg_hbm, wg_s, sem_f.at[0])
    cp_u = pltpu.make_async_copy(wu_hbm, wu_s, sem_f.at[1])
    cp_d = pltpu.make_async_copy(wd_hbm, wd_s, sem_f.at[2])

    def ln1_block(i):
        lb = _ln(x_s[pl.ds(i * TB, TB), :].astype(F32)).astype(BF16)
        for kk in range(ND):
            ln1_s[kk, pl.ds(i * TB // 2, TB // 2), :] = _pack(lb[:, kk * 128:(kk + 1) * 128])

    def k_block(i):
        rows = pl.ds(i * TB // 2, TB // 2)
        lb = _cat([_unpack(ln1_s[kk, rows, :]) for kk in range(ND)])
        wk = _cat([w_s[ND + j] for j in range(ND)])
        k = jnp.dot(lb, wk, preferred_element_type=F32)
        for a in range(ND):
            k_s[a, rows, :] = _pack(k[:, a * 128:(a + 1) * 128].astype(BF16))

    def transpose_weights(slab0, dst0):
        for kk in range(ND):
            for j in range(ND):
                tile = w_s[slab0 + j, pl.ds(kk * 128, 128), :]
                wt_s[kk, pl.ds((dst0 + j * 128) // 2, 64), :] = _pack(tile.T)

    nblk = S // TB
    cp_x[0].start()
    start_slabs(wqkv_hbm, D, w_s, ND, sem_w.at[1])
    cp_x[1].start()
    cp_x[0].wait()
    cp_x[2].start()
    ln1_block(0)
    wait_slabs(w_s, ND, sem_w.at[1])
    for i in range(nblk):
        if i + 1 < len(x_pieces):
            cp_x[i + 1].wait()
        if i + 3 < len(x_pieces):
            cp_x[i + 3].start()
        if i == 1:
            start_slabs(wqkv_hbm, 0, w_s, 0, sem_w.at[0])
        if i == 2:
            start_slabs(wqkv_hbm, 2 * D, w_s, 2 * ND, sem_w.at[2])
        if i == nblk - 2:
            wait_slabs(w_s, 0, sem_w.at[0])
            wait_slabs(w_s, 2 * ND, sem_w.at[2])
        k_block(i)
        if i + 1 < nblk:
            ln1_block(i + 1)
    transpose_weights(0, 0)
    transpose_weights(2 * ND, D)
    start_slabs(wo_hbm, 0, wo_s, 0, sem_w.at[3])
    cp_wr.start()
    cp_g.start()
    cp_u.start()
    cp_d.start()

    def qv_body(i, carry):
        cols = _rows(i * PB, PB, PB)
        half = _rows(i * (PB // 2), PB // 2, PB // 2)
        lb = _cat([_unpack(ln1_s[kk, half, :]) for kk in range(ND)])
        wq = _cat([_unpack(wt_s[kk, 0:D // 2, :]) for kk in range(ND)])
        qt_s[:, cols] = lax.dot_general(wq, lb, NT, preferred_element_type=F32) * QK_SCALE
        wv = _cat([_unpack(wt_s[kk, D // 2:D, :]) for kk in range(ND)])
        vt_s[:, cols] = _round(lax.dot_general(wv, lb, NT, preferred_element_type=F32))
        lane = lax.broadcasted_iota(jnp.int32, (PB // 2, 128), 1)
        extra = None
        for h, dst in SPECIAL:
            a, split = (h * DH) // 128, (h * DH) % 128
            both = jnp.where(lane >= split, k_s[a, half, :], k_s[a + 1, half, :])
            moved = pltpu.roll(both, (dst - split) % 128, 1)
            extra = moved if extra is None else jnp.where(lane >= dst, moved, extra)
        k_s[ND, half, :] = extra
        return carry

    lax.fori_loop(0, S // PB, qv_body, 0)

    def masked_q(wq0, off_q, q0, n):
        q = qt_s[pl.ds(wq0, 128), pl.ds(q0, n)]
        return jnp.where(_row_mask((128, n), off_q), q, 0.0).astype(BF16)

    def v_window(w0, off_v, k0, n):
        return jnp.where(_row_mask((VR, n), off_v), vt_s[pl.ds(w0, VR), pl.ds(k0, n)], 1.0)

    def finish(acc, w0, off_v, q0, live=True):
        n = acc.shape[1]
        mask = _row_mask((VR, n), off_v)
        l = jnp.sum(jnp.where(mask, 0.0, acc), axis=0, keepdims=True) * (1.0 / (VR - DH))
        o = acc * (1.0 / l)
        if live is not True:
            row = lax.broadcasted_iota(jnp.int32, (VR, n), 0)
            mask = (row >= jnp.where(live, off_v, VR)) & (row < off_v + DH)
        pltpu.store(ot_s.at[pl.ds(w0, VR), pl.ds(q0, n)], o, mask=mask)
        return o, l

    def unsafe_count(o, l):
        bad = jnp.where((jnp.abs(o) <= BIG) & (l >= L_LO) & (l <= L_HI), 0.0, 1.0)
        bad = bad[0:8] + bad[8:16] + bad[16:24]
        out = bad[:, 0:128]
        for j in range(1, NQ // 128):
            out = out + bad[:, j * 128:(j + 1) * 128]
        return out

    def finish_carried(i, acc, live):
        _, _, _, w0, off_v = _head_geom(i * HPB + HPB - 1)
        o, l = finish(acc, w0, off_v, S - NQ, live)
        return jnp.where(live, unsafe_count(o, l), 0.0)

    def fast_body(i, carry):
        bad, acc_prev = carry
        bad = bad + finish_carried(jnp.maximum(i - 1, 0), acc_prev, i > 0)
        geom = [_head_geom(i * HPB + hh) for hh in range(HPB)]
        steps = [(hh, j, c) for hh in range(HPB) for j in range(S // NQ) for c in range(S // KC)]
        n = len(steps)
        q_cache, probs, accs = {}, {}, {}
        state = {"bad": bad, "next": 0}

        def scores(hh, j, c):
            kt, wq0, off_q, _, _ = geom[hh]
            if (hh, j) not in q_cache:
                q_cache[(hh, j)] = masked_q(wq0, off_q, j * NQ, NQ)
            k = _unpack(k_s[kt, pl.ds(c * KC // 2, KC // 2), :])
            return jnp.dot(k, q_cache[(hh, j)], preferred_element_type=F32)

        def accumulate():
            t = state["next"]
            state["next"] = t + 1
            hh, j, c = steps[t]
            _, _, _, w0, off_v = geom[hh]
            r = lax.dot_general(v_window(w0, off_v, c * KC, KC), probs.pop(t), NN, preferred_element_type=F32)
            accs[j] = r if c == 0 else accs[j] + r
            if c == S // KC - 1 and t != n - 1:
                o, l = finish(accs.pop(j), w0, off_v, j * NQ)
                state["bad"] = state["bad"] + unsafe_count(o, l)

        probs[0] = jnp.exp2(scores(*steps[0])).astype(BF16)
        for t in range(n - 1):
            s = scores(*steps[t + 1])
            if t < n - 1 - TAIL:
                accumulate()
            probs[t + 1] = jnp.exp2(s).astype(BF16)
        while state["next"] < n:
            accumulate()
        return state["bad"], accs.pop(S // NQ - 1)

    nit = H // HPB
    bad, acc_last = lax.fori_loop(0, nit, fast_body, (jnp.zeros((8, 128), F32), jnp.ones((VR, NQ), F32)))
    bad = bad + finish_carried(nit - 1, acc_last, True)

    @pl.when(jnp.max(bad) > 0.0)
    def _():
        def slow_body(i, carry):
            h = i // (S // NQ)
            q0 = pl.multiple_of((i % (S // NQ)) * NQ, NQ)
            kt, wq0, off_q, w0, off_v = _head_geom(h)
            q = masked_q(wq0, off_q, q0, NQ)

            def key_body(c, mc):
                m, acc = mc
                k = _unpack(k_s[kt, _rows(c * (KC // 2), KC // 2, KC // 2), :])
                s = jnp.dot(k, q, preferred_element_type=F32)
                m_new = jnp.maximum(m, jnp.max(s, axis=0, keepdims=True))
                p = jnp.exp2(s - m_new).astype(BF16)
                v = v_window(w0, off_v, pl.multiple_of(c * KC, KC), KC)
                acc = acc * jnp.exp2(m - m_new) + lax.dot_general(v, p, NN, preferred_element_type=F32)
                return m_new, acc

            init = (jnp.full((1, NQ), -jnp.inf, F32), jnp.zeros((VR, NQ), F32))
            _, acc = lax.fori_loop(0, S // KC, key_body, init)
            finish(acc, w0, off_v, q0)
            return carry

        lax.fori_loop(0, H * (S // NQ), slow_body, 0)

    wait_slabs(wo_s, 0, sem_w.at[3])
    cp_wr.wait()
    wr = wr_s[...].reshape(1, D).astype(F32)
    sub = lax.broadcasted_iota(jnp.int32, (8, 1), 0)
    best_key = jnp.full((8, 1), -jnp.inf, F32)
    best_r = jnp.full((8, 1), jnp.nan, F32)
    best_i = sub
    for i in range(S // EB):
        rows = pl.ds(i * EB, EB)
        wo = _cat([wo_s[j] for j in range(ND)])
        attn = lax.dot_general(ot_s[:, rows].astype(BF16), wo, TN, preferred_element_type=F32)
        h = x_s[rows, :].astype(F32) + attn
        l2 = _ln(h)
        ln2_s[rows, :] = l2.astype(BF16)
        out_s[rows, :] = (h + l2).astype(BF16)
        r = _round(jnp.sum(l2 * wr, axis=-1, keepdims=True))
        key = jnp.where(r != r, -jnp.inf, r)
        for g in range(EB // 8):
            take = key[g * 8:(g + 1) * 8] > best_key
            best_key = jnp.where(take, key[g * 8:(g + 1) * 8], best_key)
            best_r = jnp.where(take, r[g * 8:(g + 1) * 8], best_r)
            best_i = jnp.where(take, sub + (i * EB + g * 8), best_i)
        if (i + 1) * EB % OB == 0:
            r0 = (i + 1) * EB - OB
            pltpu.make_async_copy(out_s.at[pl.ds(r0, OB), :], out_hbm.at[pl.ds(r0, OB), :], sem_o.at[0]).start()

    top = jnp.max(best_key, axis=0, keepdims=True)
    idx_v = jnp.min(jnp.where(best_key == top, best_i, S - 1), axis=0, keepdims=True)
    r_sel = jnp.sum(jnp.where(best_i == idx_v, best_r, 0.0), axis=0, keepdims=True)
    idx = idx_v[0, 0]
    base = pl.multiple_of((idx // 16) * 16, 16)
    sel = lax.broadcasted_iota(jnp.int32, (16, D), 0) == idx - base
    tile = ln2_s[pl.ds(base, 16), :].astype(F32)
    xs = jnp.sum(jnp.where(sel, tile, 0.0), axis=0, keepdims=True)
    xs = jnp.broadcast_to(xs, (16, D)).astype(BF16)
    cp_g.wait()
    cp_u.wait()
    cp_d.wait()
    gate = _round(jnp.dot(xs, wg_s[...], preferred_element_type=F32))
    up = _round(jnp.dot(xs, wu_s[...], preferred_element_type=F32))
    act = (_round(gate * jax.nn.sigmoid(gate)) * up).astype(BF16)
    y = jnp.dot(act, wd_s[...], preferred_element_type=F32) * jax.nn.sigmoid(r_sel)
    old = out_s[pl.ds(base, 16), :].astype(F32)
    fix_s[...] = jnp.where(sel, old + y, old).astype(BF16)
    pltpu.make_async_copy(out_s, out_hbm, sem_o.at[0]).wait()
    cp_fix = pltpu.make_async_copy(fix_s, out_hbm.at[pl.ds(base, 16), :], sem_o.at[1])
    cp_fix.start()
    cp_fix.wait()


def _block(interpret=False):
    hbm = pl.BlockSpec(memory_space=pl.ANY)
    return pl.pallas_call(
        _kernel,
        out_shape=jax.ShapeDtypeStruct((S, D), BF16),
        in_specs=[hbm] * 7,
        out_specs=hbm,
        scratch_shapes=[
            pltpu.VMEM((S, D), BF16),
            pltpu.VMEM((3 * ND, D, 128), BF16),
            pltpu.VMEM((ND, D, 128), BF16),
            pltpu.VMEM((D,), BF16),
            pltpu.VMEM((D, F), BF16),
            pltpu.VMEM((D, F), BF16),
            pltpu.VMEM((F, D), BF16),
            pltpu.VMEM((S, D), BF16),
            pltpu.VMEM((16, D), BF16),
            pltpu.VMEM((ND, S // 2, 128), U32),
            pltpu.VMEM((ND, D, 128), U32),
            pltpu.VMEM((ND + 1, S // 2, 128), U32),
            pltpu.VMEM((D, S), F32),
            pltpu.VMEM((D, S), F32),
            pltpu.VMEM((D, S), F32),
            pltpu.VMEM((S, D), BF16),
            pltpu.SemaphoreType.DMA((NSMALL + 1,)),
            pltpu.SemaphoreType.DMA((5,)),
            pltpu.SemaphoreType.DMA((3,)),
            pltpu.SemaphoreType.DMA((2,)),
        ],
        compiler_params=pltpu.CompilerParams(vmem_limit_bytes=100 * 2 ** 20),
        interpret=interpret,
        name="mha_mod_block",
    )


@jax.jit
def pallas_sequential_preLN__mha_block__moe_arch_mod__prompt_kernel(
    A_x: jax.Array,
    A_wqkv: jax.Array,
    A_wo: jax.Array,
    B_x: jax.Array,
    B_w_r: jax.Array,
    B_w_gate: jax.Array,
    B_w_up: jax.Array,
    B_w_down: jax.Array,
):
    del B_x
    out = _block()(A_x.reshape(S, D), A_wqkv, A_wo, B_w_r, B_w_gate, B_w_up, B_w_down)
    return out.reshape(1, S, D)
```
